```python
import jax
import jax.numpy as jnp

def _softmax(x, axis=-1):
    return jax.nn.softmax(x, axis=axis)
def _gelu(x):
    return jax.nn.gelu(x, approximate=True)
def _silu(x):
    return jax.nn.silu(x)
def _sigmoid(x):
    return jax.nn.sigmoid(x)
def _layernorm(x, axis=-1, eps=1e-5):
    m = jnp.mean(x, axis=axis, keepdims=True)
    v = jnp.var(x, axis=axis, keepdims=True)
    return (x - m) / jnp.sqrt(v + eps)
def _scatter_add(tgt, idx, src, axis=0):
    return tgt.at[idx].add(src)
def _segment_sum(src, seg, n):
    return jax.ops.segment_sum(src, seg, n)
class _Rng:
    def __init__(self, key):
        self._k = key
    def _next(self):
        self._k, sub = jax.random.split(self._k)
        return sub
    def normal(self, shape):
        return jax.random.normal(self._next(), shape, dtype=jnp.bfloat16)
    def randint(self, lo, hi, shape):
        return jax.random.randint(self._next(), shape, lo, hi, dtype=jnp.int32)
    def uniform(self, shape, lo=0.0, hi=1.0):
        return jax.random.uniform(self._next(), shape, jnp.bfloat16, lo, hi)
    def permutation(self, n):
        return jax.random.permutation(self._next(), n)


kernel_name = 'standalone__gqa_softmax__near_ridge'

def setup_inputs():
    _rng = _Rng(jax.random.key(int.from_bytes(__import__("os").urandom(4), "little")))
    _w = (lambda a: (lambda t: t.astype(jnp.bfloat16) if jnp.issubdtype(t.dtype, jnp.floating) else t)(jnp.asarray(a)))
    B, Hq, Hkv, Sq, Sk, D = 16, 32, 32, 848, 512, 192
    return {
        "q": _w((lambda *s: _rng.normal(s) * 0.05)(B, Hq, Sq, D)),
        "k": _w((lambda *s: _rng.normal(s) * 0.05)(B, Hkv, Sk, D)),
        "v": _w((lambda *s: _rng.normal(s) * 0.05)(B, Hkv, Sk, D)),
    }

def reference(q, k, v):
    B, Hq, Sq, D = q.shape
    Hkv = k.shape[1]
    rep = Hq // Hkv
    k = jnp.repeat(k, rep, axis=1)
    v = jnp.repeat(v, rep, axis=1)
    scale = D ** -0.5
    scores = jnp.einsum("bhqd,bhkd->bhqk", q, k) * scale
    p = _softmax(scores, axis=-1)
    return jnp.einsum("bhqk,bhkd->bhqd", p, v)
```

```python
import functools

import jax
import jax.numpy as jnp
import jax.experimental.pallas as pl
import jax.experimental.pallas.tpu as pltpu

_LOG2E = 1.4426950408889634
_HEADS_PER_STEP = 4


def _attention_kernel(qT_ref, kT_ref, vT_ref, oT_ref, *, c):
    for h in range(qT_ref.shape[0]):
        sT = jax.lax.dot_general(
            kT_ref[h], qT_ref[h], (((0,), (0,)), ((), ())),
            preferred_element_type=jnp.float32)
        m = jnp.max(sT, axis=0, keepdims=True)
        p = jnp.exp2((sT - m) * c)
        l = jnp.sum(p, axis=0, keepdims=True)
        o = jnp.dot(vT_ref[h], p.astype(jnp.bfloat16),
                    preferred_element_type=jnp.float32)
        oT_ref[h] = (o * (1.0 / l)).astype(oT_ref.dtype)


@jax.jit
def pallas_standalone__gqa_softmax__near_ridge_kernel(
    q: jax.Array,
    k: jax.Array,
    v: jax.Array,
):
    B, H, Sq, D = q.shape
    Sk = k.shape[2]
    hb = _HEADS_PER_STEP
    qT = jnp.swapaxes(q, 2, 3).reshape(B * H, D, Sq)
    kT = jnp.swapaxes(k, 2, 3).reshape(B * H, D, Sk)
    vT = jnp.swapaxes(v, 2, 3).reshape(B * H, D, Sk)
    oT = pl.pallas_call(
        functools.partial(_attention_kernel, c=D ** -0.5 * _LOG2E),
        grid=(B * H // hb,),
        in_specs=[
            pl.BlockSpec((hb, D, Sq), lambda i: (i, 0, 0)),
            pl.BlockSpec((hb, D, Sk), lambda i: (i, 0, 0)),
            pl.BlockSpec((hb, D, Sk), lambda i: (i, 0, 0)),
        ],
        out_specs=pl.BlockSpec((hb, D, Sq), lambda i: (i, 0, 0)),
        out_shape=jax.ShapeDtypeStruct((B * H, D, Sq), q.dtype),
        compiler_params=pltpu.CompilerParams(
            dimension_semantics=("parallel",),
            vmem_limit_bytes=100 * 1024 * 1024,
        ),
    )(qT, kT, vT)
    return jnp.swapaxes(oT.reshape(B, H, D, Sq), 2, 3)
```

```python
import functools

import jax
import jax.numpy as jnp
import jax.experimental.pallas as pl
import jax.experimental.pallas.tpu as pltpu

_LOG2E = 1.4426950408889634
_HEADS_PER_STEP = 8
_NN = (((1,), (0,)), ((), ()))
_NT = (((1,), (1,)), ((), ()))


def _dot(a, b, dims=_NN):
    return jax.lax.dot_general(a, b, dims, preferred_element_type=jnp.float32)


def _attention_kernel(qT_ref, kT_ref, vT_ref, oT_ref, *, c):
    sq = qT_ref.shape[-1]
    main = (sq // 128) * 128
    for h in range(qT_ref.shape[0]):
        kT, vT = kT_ref[h], vT_ref[h]
        s_tail = _dot(qT_ref[h, :, main:].T, kT)
        sT = _dot(kT.T, qT_ref[h, :, :main])

        p = jnp.exp2((s_tail - jnp.max(s_tail, axis=1, keepdims=True)) * c)
        p = (p * (1.0 / jnp.sum(p, axis=1, keepdims=True))).astype(vT.dtype)
        oT_ref[h, :128, main:] = _dot(p, vT[:128], _NT).T.astype(oT_ref.dtype)
        oT_ref[h, 128:, main:] = _dot(vT[128:], p, _NT).astype(oT_ref.dtype)

        pT = jnp.exp2((sT - jnp.max(sT, axis=0, keepdims=True)) * c)
        inv = 1.0 / jnp.sum(pT, axis=0, keepdims=True)
        oT_ref[h, :, :main] = (_dot(vT, pT.astype(vT.dtype)) * inv).astype(
            oT_ref.dtype)


@jax.jit
def pallas_standalone__gqa_softmax__near_ridge_kernel(
    q: jax.Array,
    k: jax.Array,
    v: jax.Array,
):
    B, H, Sq, D = q.shape
    Sk = k.shape[2]
    hb = _HEADS_PER_STEP
    qT = jnp.swapaxes(q, 2, 3).reshape(B * H, D, Sq)
    kT = jnp.swapaxes(k, 2, 3).reshape(B * H, D, Sk)
    vT = jnp.swapaxes(v, 2, 3).reshape(B * H, D, Sk)
    oT = pl.pallas_call(
        functools.partial(_attention_kernel, c=D ** -0.5 * _LOG2E),
        grid=(B * H // hb,),
        in_specs=[
            pl.BlockSpec((hb, D, Sq), lambda i: (i, 0, 0)),
            pl.BlockSpec((hb, D, Sk), lambda i: (i, 0, 0)),
            pl.BlockSpec((hb, D, Sk), lambda i: (i, 0, 0)),
        ],
        out_specs=pl.BlockSpec((hb, D, Sq), lambda i: (i, 0, 0)),
        out_shape=jax.ShapeDtypeStruct((B * H, D, Sq), q.dtype),
        compiler_params=pltpu.CompilerParams(
            dimension_semantics=("parallel",),
            vmem_limit_bytes=100 * 1024 * 1024,
            flags={"XLA_TPU_FORCE_LP_LLO_SCHEDULER": True},
        ),
    )(qT, kT, vT)
    return jnp.swapaxes(oT.reshape(B, H, D, Sq), 2, 3)
```

```python
import functools

import jax
import jax.numpy as jnp
import jax.experimental.pallas as pl
import jax.experimental.pallas.tpu as pltpu

_LOG2E = 1.4426950408889634
_LANES = 128
_GROUP = 16
_PIECE = 2
_LAG = 5
_FIRST_TAIL_POS = 2

_NN = (((1,), (0,)), ((), ()))
_NT = (((1,), (1,)), ((), ()))


def _dot(a, b, dims=_NN):
    return jax.lax.dot_general(a, b, dims, preferred_element_type=jnp.float32)


def _attend(q_ref, k_ref, v_ref, o_ref, k_first_ref, k_next_ref, c):
    n_heads, _, sq = q_ref.shape
    main = sq // _LANES * _LANES
    dtype = o_ref.dtype

    tiles = []
    for h in range(n_heads):
        head = [(h, start) for start in range(0, main, _LANES)]
        head.insert(_FIRST_TAIL_POS if h == 0 else 0, (h, main))
        tiles += head

    keys = {}

    def scores(h, start):
        if start == main:
            return _dot(q_ref[h, :, main:].T, k_ref[h])
        if h not in keys:
            keys[h] = k_first_ref[...] if h == 0 else k_ref[h].T
        return _dot(keys[h], q_ref[h, :, start:start + _LANES])

    def output(h, start, s):
        axis = 1 if start == main else 0
        p = jnp.exp2((s - jnp.max(s, axis=axis, keepdims=True)) * c)
        inv = 1.0 / jnp.sum(p, axis=axis, keepdims=True)
        if start == main:
            p = (p * inv).astype(v_ref.dtype)
            low = _dot(p, v_ref[h, :_LANES], _NT)
            high = _dot(v_ref[h, _LANES:], p, _NT)
            o_ref[h, :_LANES, main:] = low.astype(dtype).T
            o_ref[h, _LANES:, main:] = high.astype(dtype)
        else:
            o = _dot(v_ref[h], p.astype(v_ref.dtype)) * inv
            o_ref[h, :, start:start + _LANES] = o.astype(dtype)

    pending = {}
    for i in range(len(tiles) + _LAG):
        if i < len(tiles):
            pending[i] = scores(*tiles[i])
        if i == len(tiles) // 2:
            k_next_ref[...] = k_ref[n_heads].T
        if i >= _LAG:
            output(*tiles[i - _LAG], pending.pop(i - _LAG))


def _kernel(q_hbm, k_hbm, v_hbm, o_hbm, q_buf, k_buf, v_buf, o_buf, kt_buf,
            sem, piece_sem, *, c):
    G, S = _GROUP, _PIECE
    n_pieces = G // S
    last = q_hbm.shape[0] // G - 1
    copy = pltpu.make_async_copy

    def group_in(g, slot, n_k):
        return [
            copy(src.at[pl.ds(g * G, n)], dst.at[slot, pl.ds(0, n)],
                 sem.at[t, slot])
            for t, (src, dst, n) in enumerate(
                ((q_hbm, q_buf, G), (k_hbm, k_buf, n_k), (v_hbm, v_buf, G)))
        ]

    def piece_in(g, j, sems, sem_slot):
        return [
            copy(src.at[pl.ds(g * G + j * S + d, S)],
                 dst.at[g, pl.ds(j * S + d, S)], sems.at[t, sem_slot])
            for t, (src, dst, d) in enumerate(
                ((q_hbm, q_buf, 0), (k_hbm, k_buf, 1), (v_hbm, v_buf, 0)))
        ]

    def group_out(g, slot):
        return copy(o_buf.at[slot], o_hbm.at[pl.ds(g * G, G)], sem.at[3, slot])

    def start(copies):
        for x in copies:
            x.start()

    def wait(copies):
        for x in copies:
            x.wait()

    k_head0 = copy(k_hbm.at[pl.ds(0, 1)], k_buf.at[0, pl.ds(0, 1)],
                   piece_sem.at[3, 0])
    k_head0.start()
    start(piece_in(0, 0, piece_sem, 0))
    k_head0.wait()
    kt_buf[0] = k_buf[0, 0].T

    def small_block(phase, j):
        parity = j % 2

        @pl.when(phase == 0)
        def _():
            wait(piece_in(0, j, piece_sem, parity))

            @pl.when(j + 1 < n_pieces)
            def _():
                start(piece_in(0, j + 1, piece_sem, 1 - parity))

            start(piece_in(1, j, sem, 1))

        def view(ref, n):
            return ref.at[phase, pl.ds(j * S, n)]

        _attend(view(q_buf, S), view(k_buf, S + 1), view(v_buf, S),
                view(o_buf, S), kt_buf.at[parity], kt_buf.at[1 - parity], c)

        @pl.when(phase == 1)
        def _():
            copy(view(o_buf, S), o_hbm.at[pl.ds(last * G + j * S, S)],
                 sem.at[3, 1]).start()

    def big_block(g, carry):
        slot = g % 2
        wait(group_in(g, slot, G + 1))

        @pl.when(g + 1 < last)
        def _():
            start(group_in(g + 1, 1 - slot, G + 1))

        @pl.when(g + 1 == last)
        def _():
            start(group_in(last, 1, G))

        @pl.when(g >= 2)
        def _():
            group_out(g - 2, slot).wait()

        _attend(q_buf.at[slot], k_buf.at[slot], v_buf.at[slot], o_buf.at[slot],
                kt_buf.at[1 - slot], kt_buf.at[slot], c)
        group_out(g, slot).start()
        return carry

    def run_phase(phase, carry):
        @pl.when(phase == 0)
        def _():
            copy(k_hbm.at[pl.ds(G, 1)], k_buf.at[1, pl.ds(0, 1)],
                 sem.at[1, 1]).start()

        @pl.when(phase == 1)
        def _():
            wait(group_in(last, 1, G))
            group_out(last - 2, 1).wait()

        jax.lax.fori_loop(0, n_pieces, lambda j, _: small_block(phase, j), None)

        @pl.when(phase == 0)
        def _():
            group_out(0, 0).start()

        jax.lax.fori_loop(1, jnp.where(phase == 0, last, 1), big_block, None)
        return carry

    jax.lax.fori_loop(0, 2, run_phase, None)
    group_out(last - 1, 0).wait()
    group_out(last, 1).wait()


@jax.jit
def pallas_standalone__gqa_softmax__near_ridge_kernel(
    q: jax.Array,
    k: jax.Array,
    v: jax.Array,
):
    B, H, Sq, D = q.shape
    Sk = k.shape[2]
    n, G = B * H, _GROUP
    assert k.shape == v.shape == (B, H, Sk, D)
    assert n % (2 * G) == 0 and n >= 4 * G and (G // _PIECE) % 2 == 0
    assert Sq % _LANES and Sq // _LANES >= _FIRST_TAIL_POS and D > _LANES

    qT = jnp.swapaxes(q, 2, 3).reshape(n, D, Sq)
    kT = jnp.swapaxes(k, 2, 3).reshape(n, D, Sk)
    vT = jnp.swapaxes(v, 2, 3).reshape(n, D, Sk)
    oT = pl.pallas_call(
        functools.partial(_kernel, c=D ** -0.5 * _LOG2E),
        in_specs=[pl.BlockSpec(memory_space=pl.ANY)] * 3,
        out_specs=pl.BlockSpec(memory_space=pl.ANY),
        out_shape=jax.ShapeDtypeStruct((n, D, Sq), q.dtype),
        scratch_shapes=[
            pltpu.VMEM((2, G, D, Sq), q.dtype),
            pltpu.VMEM((2, G + 1, D, Sk), k.dtype),
            pltpu.VMEM((2, G, D, Sk), v.dtype),
            pltpu.VMEM((2, G, D, Sq), q.dtype),
            pltpu.VMEM((2, Sk, D), k.dtype),
            pltpu.SemaphoreType.DMA((4, 2)),
            pltpu.SemaphoreType.DMA((4, 2)),
        ],
        compiler_params=pltpu.CompilerParams(
            vmem_limit_bytes=100 * 1024 * 1024,
            disable_bounds_checks=True,
            flags={"XLA_TPU_FORCE_LP_LLO_SCHEDULER": True},
        ),
    )(qT, kT, vT)
    return jnp.swapaxes(oT.reshape(B, H, D, Sq), 2, 3)
```
